```python
import os as _os
_os.environ.setdefault("JAX_PLATFORMS", "cpu")
import jax
import jax.numpy as jnp

def _softmax(x, axis=-1):
    return jax.nn.softmax(x, axis=axis)
def _gelu(x):
    return jax.nn.gelu(x, approximate=True)
def _silu(x):
    return jax.nn.silu(x)
def _sigmoid(x):
    return jax.nn.sigmoid(x)
def _layernorm(x, axis=-1, eps=1e-5):
    m = jnp.mean(x, axis=axis, keepdims=True)
    v = jnp.var(x, axis=axis, keepdims=True)
    return (x - m) / jnp.sqrt(v + eps)
def _scatter_add(tgt, idx, src, axis=0):
    return tgt.at[idx].add(src)
def _segment_sum(src, seg, n):
    return jax.ops.segment_sum(src, seg, n)
class _Rng:
    def __init__(self, key):
        self._k = key
    def _next(self):
        self._k, sub = jax.random.split(self._k)
        return sub
    def normal(self, shape):
        return jax.random.normal(self._next(), shape, dtype=jnp.bfloat16)
    def randint(self, lo, hi, shape):
        return jax.random.randint(self._next(), shape, lo, hi, dtype=jnp.int32)
    def uniform(self, shape, lo=0.0, hi=1.0):
        return jax.random.uniform(self._next(), shape, jnp.bfloat16, lo, hi)
    def permutation(self, n):
        return jax.random.permutation(self._next(), n)


kernel_name = 'parallel_sum__grouped_kv_mqa__dense_activation_silu__prompt'

def setup_inputs():
    _rng = _Rng(jax.random.key(int.from_bytes(__import__("os").urandom(4), "little")))
    _w = (lambda a: (lambda t: t.astype(jnp.bfloat16) if jnp.issubdtype(t.dtype, jnp.floating) else t)(jnp.asarray(a)))
    def _A_setup():
        B, S, D, H = 1, 2048, 512, 32
        Dh = D // H
        return {
            "x": _w((lambda *s: _rng.normal(s) * 0.05)(B, S, D)),
            "wq": _w((lambda *s: _rng.normal(s) * 0.05)(D, H * Dh)),
            "wk": _w((lambda *s: _rng.normal(s) * 0.05)(D, Dh)),
            "wv": _w((lambda *s: _rng.normal(s) * 0.05)(D, Dh)),
            "wo": _w((lambda *s: _rng.normal(s) * 0.05)(H * Dh, D)),
        }
    _A_in = _A_setup()

    def _B_setup():
        B, S, D, F = 1, 2048, 512, 1376
        return {
            "x": _w((lambda *s: _rng.normal(s) * 0.05)(B, S, D)),
            "w1": _w((lambda *s: _rng.normal(s) * 0.05)(D, F) * (D ** -0.5)),
            "w2": _w((lambda *s: _rng.normal(s) * 0.05)(F, D) * (F ** -0.5)),
        }
    _B_in = _B_setup()

    return {
        "A_x": _A_in["x"],
        "A_wq": _A_in["wq"],
        "A_wk": _A_in["wk"],
        "A_wv": _A_in["wv"],
        "A_wo": _A_in["wo"],
        "B_x": _B_in["x"],
        "B_w1": _B_in["w1"],
        "B_w2": _B_in["w2"],
    }

def reference(A_x, A_wq, A_wk, A_wv, A_wo, B_x, B_w1, B_w2):
    def _A_ref(x, wq, wk, wv, wo):
        B, S, D = x.shape
        H = 32
        Dh = D // H
        q = (lambda x, *d: x.transpose(*d))((x @ wq).reshape(B, S, H, Dh), 0, 2, 1, 3)
        k = x @ wk
        v = x @ wv
        scores = jnp.einsum("bhqd,bkd->bhqk", q, k) * (Dh ** -0.5)
        p = _softmax(scores, axis=-1)
        o = jnp.einsum("bhqk,bkd->bhqd", p, v)
        return (lambda x, *d: x.transpose(*d))(o, 0, 2, 1, 3).reshape(B, S, H * Dh) @ wo

    def _B_ref(x, w1, w2):
        h = jnp.einsum("bsd,df->bsf", x, w1)
        h = _silu(h)
        out = jnp.einsum("bsf,fd->bsd", h, w2)
        return out

    x = A_x
    xn = _layernorm(x, axis=-1)
    return x + _A_ref(xn, A_wq, A_wk, A_wv, A_wo) + _B_ref(xn, B_w1, B_w2)
```

```python
import jax
import jax.numpy as jnp
from jax import lax
import jax.experimental.pallas as pl
import jax.experimental.pallas.tpu as pltpu

S, D, H, DH, F = 2048, 512, 32, 16, 1376
TQ = 512
NT = TQ // 128
NC = S // 128
RT = 256
HU = 8
LEAD = 9
POS = (1, 5, 1, 5)
UPOS = tuple(sorted(set(POS)))
NU = len(UPOS)
KT = 0
SCOPES = 0
W2 = 3
PRIO = 1
LOG2E = 1.4426950408889634
SAFE_LOG2 = 60.0
f32, bf16 = jnp.float32, jnp.bfloat16
NX = S // RT

import contextlib
def scope(name):
    return jax.named_scope(name) if SCOPES else contextlib.nullcontext()


def _kernel(x_hbm, wq_hbm, wkT_ref, wvT_ref, wo_hbm, w1T_hbm, w2_hbm, o_ref,
            x_ref, wq_ref, xn_ref, qT_ref, kp_ref, kb_ref, vT_ref, oT_ref, wT_ref,
            wo_ref, w1T_ref, w2_ref, qst_ref, flag_ref, sems, xsems):
    step = pl.program_id(0)

    def weight_copies():
        return (pltpu.make_async_copy(wo_hbm, wo_ref, sems.at[0]),
                pltpu.make_async_copy(w1T_hbm, w1T_ref, sems.at[1]),
                pltpu.make_async_copy(w2_hbm, w2_ref, sems.at[2]))

    def x_copy(r):
        return pltpu.make_async_copy(x_hbm.at[pl.ds(r * RT, RT)], x_ref.at[pl.ds(r * RT, RT)],
                                     xsems.at[r])

    @pl.when(step == 0)
    def _phase_a():
      with scope('phaseA'):
        wq_cp = pltpu.make_async_copy(wq_hbm, wq_ref, sems.at[3])
        x_copy(0).start()
        wq_cp.start()
        for r in range(1, NX):
            x_copy(r).start(priority=PRIO)
        wT_ref[D:D + DH, :] = wvT_ref[...]
        wT_ref[D + DH:D + 2 * DH, :] = wkT_ref[...]
        st = dict(q=None, k=None, v=None)

        def upd(name, val):
            st[name] = val if st[name] is None else jnp.maximum(st[name], val)

        def ln(r):
            r0 = r * RT
            x = x_ref[r0:r0 + RT, :].astype(f32)
            m = jnp.mean(x, axis=-1, keepdims=True)
            xc = x - m
            var = jnp.mean(xc * xc, axis=-1, keepdims=True)
            xn_ref[r0:r0 + RT, :] = (xc * lax.rsqrt(var + 1e-5)).astype(bf16)

        def kv(r):
            r0 = r * RT
            xn = xn_ref[r0:r0 + RT, :]
            vk = lax.dot_general(wT_ref[D:D + 2 * DH, :], xn, (((1,), (1,)), ((), ())),
                                 preferred_element_type=f32)
            vb = vk[0:DH].astype(bf16)
            vT_ref[:, r0:r0 + RT] = vb
            kT = (vk[DH:2 * DH] * (DH ** -0.5 * LOG2E)).astype(bf16).astype(f32)
            kf = kT.T
            for c in range(RT // 128):
                cc = r0 // 128 + c
                blk = jnp.concatenate([kf[c * 128 + 16 * j: c * 128 + 16 * j + 16]
                                       for j in reversed(range(8))], axis=0).astype(bf16)
                kp_ref[cc * 64:cc * 64 + 64, :] = pltpu.bitcast(blk, jnp.uint32)
                sel = jnp.concatenate([kf[c * 128 + 16 * (7 - pp): c * 128 + 16 * (8 - pp)]
                                       for pp in UPOS], axis=0)
                for d in range(DH):
                    kb_ref[d, cc * 16 * NU:(cc + 1) * 16 * NU, :] = jnp.broadcast_to(
                        sel[:, d:d + 1], (16 * NU, 128))
            upd('k', jnp.sum(kT * kT, axis=0, keepdims=True))
            upd('v', jnp.abs(vb.astype(f32)))

        def qp(r):
            r0 = r * RT
            xn = xn_ref[r0:r0 + RT, :]
            q = lax.dot_general(wT_ref[0:D, :], xn, (((1,), (1,)), ((), ())),
                                preferred_element_type=f32)
            qb = q.astype(bf16)
            qT_ref[:, r0:r0 + RT] = qb
            qr = qb.astype(f32)
            q2 = qr * qr
            for h in range(H):
                upd('q', q2[h * DH:h * DH + 8] + q2[h * DH + 8:(h + 1) * DH])

        with scope('w0x'):
            x_copy(0).wait()
        with scope('w0q'):
            wq_cp.wait()
        wT_ref[0:D, :] = wq_ref[...].T
        ln(0)
        with scope('w1'):
          for r in range(1, W2):
            x_copy(r).wait()
        for r in range(1, W2):
            ln(r)
            kv(r - 1)
            if r >= 2:
                qp(r - 2)
        with scope('w2'):
          for r in range(W2, NX):
            x_copy(r).wait()
        for cp in weight_copies():
            cp.start()
        for r in range(W2, NX):
            ln(r)
            kv(r - 1)
            qp(r - 2)
        kv(NX - 1)
        qp(NX - 2)
        qp(NX - 1)
        bound2 = jnp.max(jnp.sum(st['q'], axis=0, keepdims=True)) * jnp.max(st['k'])
        vm = jnp.max(st['v'])
        ok = (bound2 <= SAFE_LOG2 * SAFE_LOG2) & (vm <= 2.0 ** 40) & (vm >= 2.0 ** -30)
        flag_ref[0] = jnp.where(ok, 1, 0).astype(jnp.int32)

    col0 = pl.multiple_of(step * TQ, TQ)

    def kpiece(c, pp):
        r = (128 * c + 16 * pp) // 2
        return pltpu.bitcast(kp_ref[r:r + 8, :], bf16)

    mseq = [[(c, pp) for c in range(NC) for pp in range(8) if pp != POS[t]] for t in range(NT)]
    nmp = 7 * NC

    def fast_body(hh, carry):
        qs, r0s = [], []
        for u in range(HU):
            r0 = pl.multiple_of((hh * HU + u) * DH, DH)
            r0s.append(r0)
            qs.append(qT_ref[pl.ds(r0, DH), pl.ds(col0, TQ)])
            qst_ref[u] = qs[u].astype(f32)
        acc, l8, piece = {}, {}, {}

        def addl(u, t, pr):
            l8[(u, t)] = pr if (u, t) not in l8 else l8[(u, t)] + pr

        def vpiece(u, t, c):
            row = 16 * (NU * c + UPOS.index(POS[t]))
            a = None
            for d in range(DH):
                kb = kb_ref[d, row:row + 16, :]
                qrow = jnp.broadcast_to(qst_ref[u, d:d + 1, t * 128:(t + 1) * 128], (16, 128))
                pr = kb * qrow
                a = pr if a is None else a + pr
            return jnp.exp2(a)

        def do_s(u, t, a, b):
            lhs = jnp.concatenate([kpiece(*mseq[t][i]) for i in range(a, b)], axis=0)
            s = jnp.dot(lhs, qs[u][:, t * 128:(t + 1) * 128], preferred_element_type=f32)
            p = jnp.exp2(s)
            for i in range(a, b):
                piece[(u, t) + mseq[t][i]] = p[16 * (i - a):16 * (i - a + 1)]

        def do_p(u, t, c):
            seq = [vpiece(u, t, c) if pp == POS[t] else piece.pop((u, t, c, pp)) for pp in range(8)]
            for x in seq:
                addl(u, t, x[:8])
                addl(u, t, x[8:])
            p = jnp.concatenate(seq[::-1], axis=0).astype(bf16)
            o = jnp.dot(vT_ref[:, c * 128:(c + 1) * 128], p, preferred_element_type=f32)
            acc[(u, t)] = o if (u, t) not in acc else acc[(u, t)] + o

        done = 0
        for u in range(HU):
            for c in range(NC):
                target = min(HU * nmp, u * nmp + 7 * (c + 1) + LEAD)
                while done < target:
                    uu = done // nmp
                    e = min(target, (uu + 1) * nmp)
                    for t in range(NT):
                        do_s(uu, t, done - uu * nmp, e - uu * nmp)
                    done = e
                for t in range(NT):
                    do_p(u, t, c)
            a = jnp.concatenate([acc[(u, t)] for t in range(NT)], axis=1)
            l = jnp.sum(jnp.concatenate([l8[(u, t)] for t in range(NT)], axis=1),
                        axis=0, keepdims=True)
            oT_ref[pl.ds(r0s[u], DH), :] = (a / l).astype(bf16)
        return carry

    def slow_body(h, carry):
        r0 = pl.multiple_of(h * DH, DH)
        qh = qT_ref[pl.ds(r0, DH), pl.ds(col0, TQ)]
        kn = jnp.concatenate([kpiece(c, 7 - j) for c in range(NC) for j in range(8)], axis=0)
        s = jnp.dot(kn, qh, preferred_element_type=f32)
        m = jnp.max(s, axis=0, keepdims=True)
        p = jnp.exp2(s - m)
        l = jnp.sum(p, axis=0, keepdims=True)
        o = jnp.dot(vT_ref[...], p.astype(bf16), preferred_element_type=f32)
        oT_ref[pl.ds(r0, DH), :] = (o / l).astype(bf16)
        return carry

    safe = flag_ref[0]

    @pl.when(safe == 1)
    def _():
        with scope('attn'):
            lax.fori_loop(0, H // HU, fast_body, 0)

    @pl.when(safe != 1)
    def _():
        lax.fori_loop(0, H, slow_body, 0)

    @pl.when(step == 0)
    def _():
        for cp in weight_copies():
            cp.wait()

    with scope('dense'):
        xn_t = xn_ref[pl.ds(col0, TQ), :]
        attn = lax.dot_general(oT_ref[...], wo_ref[...], (((0,), (0,)), ((), ())),
                               preferred_element_type=f32)
        hh = lax.dot_general(xn_t, w1T_ref[...], (((1,), (1,)), ((), ())),
                             preferred_element_type=f32)
        hh = hh * jax.nn.sigmoid(hh)
        y = jnp.dot(hh.astype(bf16), w2_ref[...], preferred_element_type=f32)
        xt = x_ref[pl.ds(col0, TQ), :].astype(f32)
        o_ref[...] = (xt + attn + y).astype(o_ref.dtype)


@jax.jit
def pallas_parallel_sum__grouped_kv_mqa__dense_activation_silu__prompt_kernel(
        A_x, A_wq, A_wk, A_wv, A_wo, B_x, B_w1, B_w2):
    x = A_x.reshape(S, D)
    full = lambda shp: pl.BlockSpec(shp, lambda i: (0,) * len(shp))
    hbm = pl.BlockSpec(memory_space=pl.ANY)
    out = pl.pallas_call(
        _kernel,
        grid=(S // TQ,),
        in_specs=[hbm, hbm, full((DH, D)), full((DH, D)), hbm, hbm, hbm],
        out_specs=pl.BlockSpec((TQ, D), lambda i: (i, 0)),
        out_shape=jax.ShapeDtypeStruct((S, D), bf16),
        scratch_shapes=[
            pltpu.VMEM((S, D), bf16),
            pltpu.VMEM((D, D), bf16),
            pltpu.VMEM((S, D), bf16),
            pltpu.VMEM((D, S), bf16),
            pltpu.VMEM((S // 2, DH), jnp.uint32),
            pltpu.VMEM((DH, NC * 16 * NU, 128), f32),
            pltpu.VMEM((DH, S), bf16),
            pltpu.VMEM((D, TQ), bf16),
            pltpu.VMEM((D + 2 * DH, D), bf16),
            pltpu.VMEM((D, D), bf16),
            pltpu.VMEM((F, D), bf16),
            pltpu.VMEM((F, D), bf16),
            pltpu.VMEM((HU, DH, TQ), f32),
            pltpu.SMEM((1,), jnp.int32),
            pltpu.SemaphoreType.DMA((4,)),
            pltpu.SemaphoreType.DMA((NX,)),
        ],
        compiler_params=pltpu.CompilerParams(
            dimension_semantics=("arbitrary",),
            vmem_limit_bytes=100 * 1024 * 1024),
    )(x, A_wq, A_wk.T, A_wv.T, A_wo, B_w1.T, B_w2)
    return out.reshape(1, S, D)
```

```python
import jax
import jax.numpy as jnp
from jax import lax
import jax.experimental.pallas as pl
import jax.experimental.pallas.tpu as pltpu

S, D, H, DH, F = 2048, 512, 32, 16, 1376
TQ = 512
NT = TQ // 128
NC = S // 128
NSTEP = S // TQ
RT = 256
NX = S // RT
NF = -(-F // 128)
HU = 8
LOG2E = 1.4426950408889634
SAFE_LOG2 = 60.0
f32, bf16, u32 = jnp.float32, jnp.bfloat16, jnp.uint32

LEAD = 9
VPOS = 6
LANC = (1, 5, 3, 6)
PREP = 2
PRET = (1, 5, 9, 13, 3, 7, 11, 15)
NPH = (8, 4, 4, 4, 4, 4, 4, 4)
ND = 4
NE = 3
SELF = (14, 15)
TSPEC = '252,352,452,552,652,752,852,952,a52,b52,c52,d52'
SSPEC = '252,352,452,652,752,852,a52,b52'
NS = 8
QTK = 1
R1 = 19.0
R2 = 24.0
RO = 24.0
OPOS = 11
TIE0 = 2.0
TIE1 = 3.0
CDD = 2
NA = 80
APRE = 10
B2, B3, W2 = 1, 5, 3
KDEL = 4
LND = 2
SCOPES = 0

NPRE = len(PRET)
EXT = PRET[ND:ND + NE]
KBSLOT = {}
for _c in range(NC):
    for _t in range(NT):
        KBSLOT[(_c, VPOS, _t)] = len(KBSLOT)
    if _c in PRET + SELF:
        KBSLOT[(_c, PREP, 0)] = len(KBSLOT)
NKB = len(KBSLOT)
TODO = [(h, t, j) for j in range(NPRE) for h in range(H) for t in range(NT) if j < NPH[h % HU]]


def _not_mxu(u, c):
    ahead = PRET[:NPH[u]] + EXT + (SELF if u == HU - 1 else ())
    return [VPOS] + ([PREP] if c in ahead else [])


_FULL = [[(c, pp) for c in range(NC) for pp in range(8) if pp not in _not_mxu(u, c)]
         for u in range(HU)]
CARRY = _FULL[0][:NS]
MSEQ = [_FULL[0][NS:]] + _FULL[1:] + [CARRY]
START = [sum(len(m) for m in MSEQ[:u]) for u in range(HU + 2)]
MEND = [[START[u] + sum(1 for (cc, _) in MSEQ[u] if cc <= c) for c in range(NC)] for u in range(HU)]
TIES = {}
for _u in range(HU - 1):
    for _k, (_t, _c2) in enumerate((t, c2) for t in range(NT) for c2 in EXT):
        _c, _lp, _ht = (int(ch, 16) for ch in TSPEC.split(',')[_k])
        TIES.setdefault((_u, _ht, _c, _lp), []).append((_u + 1, _t, _c2))
for _k, (_c2, _t) in enumerate((c2, t) for c2 in SELF for t in range(NT)):
    _c, _lp, _ht = (int(ch, 16) for ch in SSPEC.split(',')[_k])
    TIES.setdefault((HU - 1, _ht, _c, _lp), []).append((HU - 1, _t, _c2))

import contextlib
def scope(name):
    return jax.named_scope(name) if SCOPES else contextlib.nullcontext()


def _lanes(t):
    return slice(t * 128, (t + 1) * 128)


def _silu(h):
    return h * pl.reciprocal(1.0 + jnp.exp2(h * -LOG2E), approx=True)


def _kernel(x_hbm, wq_hbm, wkT_hbm, wvT_hbm, wo_hbm, w1T_hbm, w2_hbm, o_hbm,
            o_ref, wkT_ref, wvT_ref, x_ref, wq_ref, xn_ref, qT_ref, kp_ref, kb_ref, vT_ref,
            oT_ref, wT_ref, wo_ref, w1T_ref, w2_ref, qst_ref, qall_ref, pre_ref, y_ref,
            carry_ref, flag_ref, sems, xsems, osems):
    step = pl.program_id(0)

    def late_copies():
        return (pltpu.make_async_copy(w1T_hbm, w1T_ref, sems.at[0]),
                pltpu.make_async_copy(w2_hbm, w2_ref, sems.at[1]),
                pltpu.make_async_copy(wo_hbm, wo_ref, sems.at[2]))

    def early_copies():
        return (pltpu.make_async_copy(wkT_hbm, wkT_ref, sems.at[3]),
                pltpu.make_async_copy(wvT_hbm, wvT_ref, sems.at[4]),
                pltpu.make_async_copy(wq_hbm, wq_ref, sems.at[5]))

    def x_copy(r):
        return pltpu.make_async_copy(x_hbm.at[pl.ds(r * RT, RT)], x_ref.at[pl.ds(r * RT, RT)],
                                     xsems.at[r])

    def o_copy(m, row0):
        return pltpu.make_async_copy(o_ref.at[:, pl.ds(m * 128, 128)],
                                     o_hbm.at[pl.ds(row0, TQ), pl.ds(m * 128, 128)], osems.at[m])

    def kpiece(c, pp):
        r = (128 * c + 16 * pp) // 2
        return pltpu.bitcast(kp_ref[r:r + 8, :], bf16)

    def keep_mask():
        return (pltpu.bitcast(wkT_ref[:, 0:128], jnp.int32) & 1) < 2

    def vscore(cache, kcache, q_ref, qi, t, c, pp, cd):
        if (qi, t) not in cache:
            rows = [jnp.broadcast_to(q_ref[qi, d:d + 1, _lanes(t)], (1, 1, 8, 128))
                    for d in range(DH)]
            cache[(qi, t)] = [jnp.concatenate(rows[d:d + cd], axis=0) if cd > 1 else rows[d]
                              for d in range(0, DH, cd)]
        slot = KBSLOT[(c, pp, t if pp == VPOS else 0)]
        if slot not in kcache:
            kv = kb_ref[slot]
            kcache[slot] = [kv[d:d + cd] for d in range(0, DH, cd)]
        a = None
        for kb, qb in zip(kcache[slot], cache[(qi, t)]):
            pr = jnp.sum(kb * qb, axis=0) if cd > 1 else kb * qb
            a = pr if a is None else a + pr
        return jnp.exp2(a).reshape(16, 128)

    def emit_pre(cache, item, blk):
        if 'keep' not in cache:
            cache['keep'] = keep_mask()
        h, t, j = item
        p = vscore(cache, cache, qall_ref, h, t, PRET[j], PREP, CDD)
        pre_ref[h, j, :, _lanes(t)] = p
        return jnp.where(cache['keep'], blk, pltpu.bitcast(p[:8] + p[8:], blk.dtype))

    @pl.when(step == 0)
    def _():
      with scope('phaseA'):
        x_copy(0).start()
        for cp in early_copies():
            cp.start()
        for r in range(1, NX):
            x_copy(r).start(priority=1)
        st = dict(q=None, k=None, v=None, pre=0)
        qc, pend = {}, []

        def upd(name, val):
            st[name] = val if st[name] is None else jnp.maximum(st[name], val)

        def ln(i):
            x = x_ref[i * 128:(i + 1) * 128, :].astype(f32)
            xc = x - jnp.mean(x, axis=-1, keepdims=True)
            var = jnp.mean(xc * xc, axis=-1, keepdims=True)
            xn = (xc * lax.rsqrt(var + 1e-5)).astype(bf16)
            xn_ref[i * 128:(i + 1) * 128, :] = xn
            return xn

        def kproc(i, kT):
            kf = kT.T
            blk = jnp.concatenate([kf[16 * j:16 * j + 16] for j in reversed(range(8))], axis=0)
            kp_ref[i * 64:i * 64 + 64, :] = pltpu.bitcast(blk.astype(bf16), u32)
            pps = [VPOS] + ([PREP] if i in PRET + SELF else [])
            sel = jnp.concatenate([blk[16 * pp:16 * pp + 16] for pp in pps], axis=0)
            s0 = KBSLOT[(i, VPOS, 0)]
            for d in range(DH):
                bc = jnp.broadcast_to(sel[:, d:d + 1], (16 * len(pps), 128))
                bc = bc.reshape(len(pps), 2, 8, 128)
                kb_ref[s0:s0 + NT + len(pps) - 1, d] = jnp.concatenate(
                    [bc[0:1]] * NT + [bc[1:]] * (len(pps) - 1), axis=0)

        def proj(i, xn):
            nb = (D + 2 * DH) // 16
            wu = wT_ref[...]
            if i >= NC - NA // APRE:
                rows = []
                for b in range(nb):
                    blk = wu[8 * b:8 * b + 8, 0:128]
                    for _ in range((b + 1) * APRE // nb - b * APRE // nb):
                        blk = emit_pre(qc, TODO[st['pre']], blk)
                        st['pre'] += 1
                    rows.append(blk)
                wu = jnp.concatenate([jnp.concatenate(rows, axis=0), wu[:, 128:]], axis=1)
            vkq = lax.dot_general(pltpu.bitcast(wu, bf16), xn, (((1,), (1,)), ((), ())),
                                  preferred_element_type=f32)
            vb = vkq[0:DH].astype(bf16)
            vT_ref[:, _lanes(i)] = vb
            kT = (vkq[DH:2 * DH] * (DH ** -0.5 * LOG2E)).astype(bf16).astype(f32)
            pend.append((i, kT))
            while len(pend) > (KDEL if i < NC - 1 else 0):
                kproc(*pend.pop(0))
            upd('k', jnp.sum(kT * kT, axis=0, keepdims=True))
            upd('v', jnp.abs(vb.astype(f32)))
            qb = vkq[2 * DH:].astype(bf16)
            qT_ref[:, _lanes(i)] = qb
            qr = qb.astype(f32)
            if i < NT:
                qall_ref[:, :, _lanes(i)] = qr.reshape(H, DH, 128)
            q2 = qr * qr
            for h in range(H):
                upd('q', q2[h * DH:h * DH + 8] + q2[h * DH + 8:(h + 1) * DH])

        x_copy(0).wait()
        ln(0)
        for cp in early_copies():
            cp.wait()
        wT_ref[0:8, :] = pltpu.bitcast(wvT_ref[...], u32)
        wT_ref[8:16, :] = pltpu.bitcast(wkT_ref[...], u32)
        wT_ref[16:, :] = pltpu.bitcast(wq_ref[...].T, u32)
        avail = RT // 128
        xns = {0: None}
        for i in range(NC):
            if i == B2:
                for r in range(1, W2):
                    x_copy(r).wait()
                avail = W2 * RT // 128
                xns = {k: None for k in xns}
            if i == B3:
                for cp in late_copies():
                    cp.start(priority=1)
                for r in range(W2, NX):
                    x_copy(r).wait()
                avail = NC
                xns = {k: None for k in xns}
            for k in range(i, min(avail, i + LND + 1)):
                if k not in xns:
                    xns[k] = ln(k)
            proj(i, xns[i] if xns[i] is not None else xn_ref[i * 128:(i + 1) * 128, :])
        assert st['pre'] == NA
        bound2 = jnp.max(jnp.sum(st['q'], axis=0, keepdims=True)) * jnp.max(st['k'])
        vm = jnp.max(st['v'])
        ok = (bound2 <= SAFE_LOG2 * SAFE_LOG2) & (vm <= 2.0 ** 40) & (vm >= 2.0 ** -30)
        flag_ref[0] = jnp.where(ok, 1, 0).astype(jnp.int32)
        for cp in late_copies():
            cp.wait()

    col0 = pl.multiple_of(step * TQ, TQ)
    nxt = pl.multiple_of(jnp.minimum(step + 1, NSTEP - 1) * TQ, TQ)

    def dense(do_o, do_f, rows0, skip=0):
        gsl = TQ // 16
        g2 = ([((k, k + 2), (m, m + 2)) for k in range(0, NF - 1, 2) for m in (0, 2)]
              + [((NF - 1, NF), (0, 4))])
        plan = []
        if do_f:
            plan += [('1', n) for n in range(NF)] + [('2', g) for g in g2]
        if do_o:
            plan[OPOS:OPOS] = [('o', m) for m in range(D // 128)]
        todo = TODO[skip:] if do_f else []
        rate = {'1': R1, '2': R2, 'o': RO}
        cum = [0.0]
        for kind, _ in plan:
            cum.append(cum[-1] + rate[kind])
        state, qc = dict(done=0), {}

        def tie(blk, gi, r):
            frac = ((cum[gi] + (cum[gi + 1] - cum[gi]) * (r + 1) / gsl - TIE0)
                    / (cum[-1] - TIE0 - TIE1))
            while state['done'] < len(todo) and state['done'] + 1 <= frac * len(todo):
                blk = emit_pre(qc, todo[state['done']], blk)
                state['done'] += 1
            return blk

        def tie_acc(a, gi):
            if not do_f:
                return a
            rows = []
            for r in range(gsl):
                rows += [tie(a[16 * r:16 * r + 8], gi, r), a[16 * r + 8:16 * r + 16]]
            return jnp.concatenate(rows, axis=0)

        if do_f:
            xu = pltpu.bitcast(xn_ref[pl.ds(rows0, TQ), :], u32)
            xres = x_ref[pl.ds(rows0, TQ), :].astype(f32)
            acc = [xres[:, _lanes(m)] for m in range(D // 128)]
        if do_o:
            o_all = oT_ref[...].T
        gs, gcat = [], {}
        for gi, (kind, arg) in enumerate(plan):
            if kind == '1':
                n0, n1 = arg * 128, min(F, (arg + 1) * 128)
                w = w1T_ref[n0:n1, :]
                if n1 - n0 < 128:
                    w = jnp.concatenate([w, jnp.zeros((128 - (n1 - n0), D), bf16)], axis=0)
                first = jnp.concatenate([tie(xu[8 * r:8 * r + 8, 0:128], gi, r)
                                         for r in range(gsl)], axis=0)
                lhs = pltpu.bitcast(jnp.concatenate([first, xu[:, 128:]], axis=1), bf16)
                gs.append(_silu(lax.dot_general(lhs, w, (((1,), (1,)), ((), ())),
                                                preferred_element_type=f32)))
            elif kind == '2':
                (ka, kb_), (ma, mb) = arg
                k0, k1 = ka * 128, min(F, kb_ * 128)
                if (ka, kb_) not in gcat:
                    gcat[(ka, kb_)] = jnp.concatenate(gs[ka:kb_], axis=1).astype(bf16)[:, :k1 - k0]
                yp = jnp.dot(gcat[(ka, kb_)], w2_ref[k0:k1, ma * 128:mb * 128],
                             preferred_element_type=f32)
                acc[ma] = tie_acc(acc[ma], gi)
                new = yp + jnp.concatenate(acc[ma:mb], axis=1)
                for m in range(ma, mb):
                    acc[m] = new[:, _lanes(m - ma)]
            else:
                op = jnp.dot(o_all, wo_ref[:, _lanes(arg)], preferred_element_type=f32)
                o_ref[:, _lanes(arg)] = (op + tie_acc(y_ref[:, _lanes(arg)], gi)).astype(bf16)
                o_copy(arg, col0).start()
        if do_f:
            y_ref[...] = jnp.concatenate(acc, axis=1)
        assert state['done'] == len(todo)

    @pl.when(step == 0)
    def _():
        with scope('ffn0'):
            dense(False, True, 0, NA)
            lhs = jnp.concatenate([kpiece(c, pp) for (c, pp) in CARRY], axis=0)
            p0 = jnp.exp2(jnp.dot(lhs, qT_ref[0:DH, 0:TQ], preferred_element_type=f32))
            carry_ref[...] = p0.reshape(NS, 16, TQ)

    def fast_body(hh, carry):
        wrap = hh == H // HU - 1
        qs, r0s = [], []
        for u in range(HU):
            r0 = pl.multiple_of((hh * HU + u) * DH, DH)
            r0s.append(r0)
            qs.append(qT_ref[pl.ds(r0, DH), pl.ds(col0, TQ)])
            qall_ref[hh * HU + u] = qT_ref[pl.ds(r0, DH), pl.ds(nxt, TQ)].astype(f32)
            qst_ref[u] = qs[u].astype(f32)
        rn = pl.multiple_of(jnp.where(wrap, 0, (hh + 1) * HU) * DH, DH)
        cn = pl.multiple_of(jnp.where(wrap, nxt, col0), TQ)
        qs.append(qT_ref[pl.ds(rn, DH), pl.ds(cn, TQ)])
        acc, lsum, piece, qc, kc = {}, {}, {}, {}, {}
        qce = {}
        keep = keep_mask()

        def get(u, t, c, pp):
            if c in PRET[:NPH[u]] and pp == PREP:
                return pre_ref[hh * HU + u, PRET.index(c), :, _lanes(t)]
            if pp == VPOS:
                return vscore(qc, {}, qst_ref, u, t, c, pp, 1)
            if u == 0 and (c, pp) in CARRY:
                return carry_ref[CARRY.index((c, pp)), :, _lanes(t)]
            return piece.pop((u, t, c, pp))

        def do_s(u, a, b):
            for cp in MSEQ[u][a:b]:
                if cp not in kc:
                    kc[cp] = kpiece(*cp)
            lhs = jnp.concatenate([kc[cp] for cp in MSEQ[u][a:b]], axis=0)
            for t in range(NT):
                p = jnp.exp2(jnp.dot(lhs, qs[u][:, _lanes(t)], preferred_element_type=f32))
                for i in range(a, b):
                    x = p[16 * (i - a):16 * (i - a + 1)]
                    if u == HU:
                        carry_ref[i, :, _lanes(t)] = x
                    else:
                        piece[(u, t) + MSEQ[u][i]] = x

        def tie(a, z):
            return jnp.concatenate([jnp.where(keep, a[:8], z), a[8:]], axis=0)

        def do_p(u, t, c):
            order = [pp for pp in range(8) if pp != VPOS]
            order.insert(LANC[t], VPOS)
            val = {}
            for k, pp in enumerate(order):
                for (u2, t2, c2) in TIES.get((u, t, c, k), []):
                    pe = vscore(qce, {}, qst_ref, u2, t2, c2, PREP, 1)
                    piece[(u2, t2, c2, PREP)] = pe
                    lsum[(u, t)] = tie(lsum[(u, t)], pe[:8] + pe[8:])
                if u == 0 and c == 0 and k == QTK:
                    z = None
                    for u2 in range(1, HU):
                        for d in (0, 8):
                            r = jnp.broadcast_to(qst_ref[u2, d:d + 1, _lanes(t)], (8, 128))
                            z = r if z is None else jnp.maximum(z, r)
                    lsum[(u, t)] = tie(lsum[(u, t)], z)
                val[pp] = x = get(u, t, c, pp)
                lsum[(u, t)] = x if (u, t) not in lsum else lsum[(u, t)] + x
            p = jnp.concatenate([val[pp] for pp in reversed(range(8))], axis=0).astype(bf16)
            o = jnp.dot(vT_ref[:, _lanes(c)], p, preferred_element_type=f32)
            acc[(u, t)] = o if (u, t) not in acc else acc[(u, t)] + o

        done = 0
        for u in range(HU):
            for c in range(NC):
                target = min(START[HU + 1], MEND[u][c] + LEAD)
                while done < target:
                    uu = max(v for v in range(HU + 1) if START[v] <= done)
                    e = min(target, START[uu + 1])
                    do_s(uu, done - START[uu], e - START[uu])
                    done = e
                for t in range(NT):
                    do_p(u, t, c)
            a = jnp.concatenate([acc[(u, t)] for t in range(NT)], axis=1)
            l = jnp.sum(jnp.concatenate([lsum[(u, t)] for t in range(NT)], axis=1),
                        axis=0, keepdims=True)
            oT_ref[pl.ds(r0s[u], DH), :] = (a / l).astype(bf16)
        assert done == START[HU + 1]
        return carry

    def slow_body(i, carry):
        r0 = pl.multiple_of((i // 2) * DH, DH)
        c0 = pl.multiple_of((i % 2) * (TQ // 2), TQ // 2)
        qh = qT_ref[pl.ds(r0, DH), pl.ds(pl.multiple_of(col0 + c0, TQ // 2), TQ // 2)]
        qall_ref[i // 2] = qT_ref[pl.ds(r0, DH), pl.ds(nxt, TQ)].astype(f32)
        kn = jnp.concatenate([kpiece(c, 7 - j) for c in range(NC) for j in range(8)], axis=0)
        s = jnp.dot(kn, qh, preferred_element_type=f32)
        p = jnp.exp2(s - jnp.max(s, axis=0, keepdims=True))
        l = jnp.sum(p, axis=0, keepdims=True)
        o = jnp.dot(vT_ref[...], p.astype(bf16), preferred_element_type=f32)
        oT_ref[pl.ds(r0, DH), pl.ds(c0, TQ // 2)] = (o / l).astype(bf16)
        return carry

    safe = flag_ref[0]

    @pl.when(safe == 1)
    def _():
        with scope('attn'):
            lax.fori_loop(0, H // HU, fast_body, 0)

    @pl.when(safe != 1)
    def _():
        lax.fori_loop(0, 2 * H, slow_body, 0)

    @pl.when(step > 0)
    def _():
        prev = pl.multiple_of(jnp.maximum(step - 1, 0) * TQ, TQ)
        for m in range(D // 128):
            o_copy(m, prev).wait()

    @pl.when(step < NSTEP - 1)
    def _():
        with scope('of'):
            dense(True, True, nxt)

    @pl.when(step == NSTEP - 1)
    def _():
        with scope('o'):
            dense(True, False, None)
        for m in range(D // 128):
            o_copy(m, col0).wait()


@jax.jit
def pallas_parallel_sum__grouped_kv_mqa__dense_activation_silu__prompt_kernel(
        A_x, A_wq, A_wk, A_wv, A_wo, B_x, B_w1, B_w2):
    hbm = pl.BlockSpec(memory_space=pl.ANY)
    out = pl.pallas_call(
        _kernel,
        grid=(NSTEP,),
        in_specs=[hbm] * 7,
        out_specs=hbm,
        out_shape=jax.ShapeDtypeStruct((S, D), bf16),
        scratch_shapes=[
            pltpu.VMEM((TQ, D), bf16),
            pltpu.VMEM((DH, D), bf16),
            pltpu.VMEM((DH, D), bf16),
            pltpu.VMEM((S, D), bf16),
            pltpu.VMEM((D, D), bf16),
            pltpu.VMEM((S, D), bf16),
            pltpu.VMEM((D, S), bf16),
            pltpu.VMEM((S // 2, DH), u32),
            pltpu.VMEM((NKB, DH, 2, 8, 128), f32),
            pltpu.VMEM((DH, S), bf16),
            pltpu.VMEM((D, TQ), bf16),
            pltpu.VMEM((D // 2 + DH, D), u32),
            pltpu.VMEM((D, D), bf16),
            pltpu.VMEM((F, D), bf16),
            pltpu.VMEM((F, D), bf16),
            pltpu.VMEM((HU, DH, TQ), f32),
            pltpu.VMEM((H, DH, TQ), f32),
            pltpu.VMEM((H, NPRE, 16, TQ), f32),
            pltpu.VMEM((TQ, D), f32),
            pltpu.VMEM((NS, 16, TQ), f32),
            pltpu.SMEM((1,), jnp.int32),
            pltpu.SemaphoreType.DMA((6,)),
            pltpu.SemaphoreType.DMA((NX,)),
            pltpu.SemaphoreType.DMA((D // 128,)),
        ],
        compiler_params=pltpu.CompilerParams(
            dimension_semantics=("arbitrary",),
            vmem_limit_bytes=100 * 1024 * 1024),
    )(A_x.reshape(S, D), A_wq, A_wk.T, A_wv.T, A_wo, B_w1.T, B_w2)
    return out.reshape(1, S, D)
```
